```python
import os as _os
_os.environ.setdefault('JAX_PLATFORMS', 'cpu')
import jax
import jax.numpy as jnp

def _softmax(x, axis=-1):
    return jax.nn.softmax(x, axis=axis)

def _gelu(x):
    return jax.nn.gelu(x, approximate=True)

def _silu(x):
    return jax.nn.silu(x)

def _sigmoid(x):
    return jax.nn.sigmoid(x)

def _layernorm(x, axis=-1, eps=1e-05):
    m = jnp.mean(x, axis=axis, keepdims=True)
    v = jnp.var(x, axis=axis, keepdims=True)
    return (x - m) / jnp.sqrt(v + eps)

def _scatter_add(tgt, idx, src, axis=0):
    return tgt.at[idx].add(src)

def _segment_sum(src, seg, n):
    return jax.ops.segment_sum(src, seg, n)

class _Rng:

    def __init__(self, key):
        self._k = key

    def _next(self):
        self._k, sub = jax.random.split(self._k)
        return sub

    def normal(self, shape):
        return jax.random.normal(self._next(), shape, dtype=jnp.bfloat16)

    def randint(self, lo, hi, shape):
        return jax.random.randint(self._next(), shape, lo, hi, dtype=jnp.int32)

    def uniform(self, shape, lo=0.0, hi=1.0):
        return jax.random.uniform(self._next(), shape, jnp.bfloat16, lo, hi)

    def permutation(self, n):
        return jax.random.permutation(self._next(), n)
kernel_name = 'adaLN_cond__spectral_gfnet__dense_activation_squared_relu__prompt'

def setup_inputs():
    _rng = _Rng(jax.random.key(int.from_bytes(__import__("os").urandom(4), "little")))
    _w = lambda a: (lambda t: t.astype(jnp.bfloat16) if jnp.issubdtype(t.dtype, jnp.floating) else t)(jnp.asarray(a))

    def _A_setup():
        B, S, D = (1, 2048, 640)
        Df = D // 2 + 1
        return {'x': _w((lambda *s: _rng.normal(s) * 0.05)(B, S, D)), 'w_r': _w((lambda *s: _rng.normal(s) * 0.2)(S, Df) * 0.02), 'w_i': _w((lambda *s: _rng.normal(s) * 0.2)(S, Df) * 0.02)}
    _A_in = _A_setup()

    def _B_setup():
        B, S, D, F = (1, 2048, 640, 1728)
        return {'x': _w((lambda *s: _rng.normal(s) * 0.05)(B, S, D)), 'w1': _w((lambda *s: _rng.normal(s) * 0.05)(D, F)), 'b1': _w((lambda *s: _rng.normal(s) * 0.05)(F)), 'w2': _w((lambda *s: _rng.normal(s) * 0.05)(F, D)), 'b2': _w((lambda *s: _rng.normal(s) * 0.05)(D))}
    _B_in = _B_setup()
    return {'A_x': _A_in['x'], 'A_w_r': _A_in['w_r'], 'A_w_i': _A_in['w_i'], 'B_x': _B_in['x'], 'B_w1': _B_in['w1'], 'B_b1': _B_in['b1'], 'B_w2': _B_in['w2'], 'B_b2': _B_in['b2'], 'c': _w((lambda *s: _rng.normal(s) * 0.2)(1, 640) * 8.0), 'w_mod': _w((lambda *s: _rng.normal(s) * 0.2)(640, 6 * 640) * 640 ** (-0.5) * 8.0)}

def reference(A_x, A_w_r, A_w_i, B_x, B_w1, B_b1, B_w2, B_b2, c, w_mod):

    def _A_ref(x, w_r, w_i):
        B, S, D = x.shape
        X = (lambda x, axes=(-2, -1): jnp.fft.rfft2(x.astype(jnp.float32), axes=axes))(x, axes=(-2, -1))
        W = w_r + 1j * w_i
        X = X * W
        y = (lambda x, s, axes=(-2, -1): jnp.fft.irfft2(x, s=s, axes=axes).astype(jnp.bfloat16))(X, (S, D), axes=(-2, -1))
        return y

    def _B_ref(x, w1, b1, w2, b2):
        h = jnp.einsum('bsd,df->bsf', x, w1) + b1
        zero = jnp.zeros_like(h)
        r = jnp.where(h > zero, h, zero)
        h = r * r
        out = jnp.einsum('bsf,fd->bsd', h, w2) + b2
        return out
    x = A_x
    mod = (_silu(c) @ w_mod).reshape(c.shape[0], 6, 1, -1)
    sa, ca, ga, sb, cb, gb = (mod[:, 0].copy(), mod[:, 1].copy(), mod[:, 2].copy(), mod[:, 3].copy(), mod[:, 4].copy(), mod[:, 5].copy())
    h = _layernorm(x, axis=-1) * (1 + ca) + sa
    x = x + ga * _A_ref(h, A_w_r, A_w_i)
    h = _layernorm(x, axis=-1) * (1 + cb) + sb
    x = x + gb * _B_ref(h, B_w1, B_b1, B_w2, B_b2)
    return x
```

```python
import functools

import numpy as np

import jax
import jax.numpy as jnp
from jax import lax
import jax.experimental.pallas as pl
import jax.experimental.pallas.tpu as pltpu

S, D, F = 2048, 640, 1728
KD = D // 2 + 1
NT = S // 128
ND = D // 128
EPS = 1e-5
X_SEM = 20
TPC = 4
NCH = NT // TPC
FH = F // 2
KT = -(-FH // 128)
UP_ROWS, DOWN_ROWS = 96, 64
UP_PACE, DOWN_PACE = 2, 2
SPLIT = 3 * UP_ROWS

bf16, f32, u32 = jnp.bfloat16, jnp.float32, jnp.uint32
_NT_DIMS = (((1,), (1,)), ((), ()))

_SIN1, _SIN2 = np.sin(2 * np.pi / 5), np.sin(4 * np.pi / 5)
_RHO = float(_SIN2 / _SIN1)
_C5 = float(np.sqrt(5.0) / 4)
_R2 = float(np.sqrt(0.5))
_C8, _S8 = float(np.cos(np.pi / 8)), float(np.sin(np.pi / 8))
_GROUP_RES = ((0, 5), (1, 9), (2, 8), (3, 7), (4, 6))


def _d_matrices():
  coef = {0: (1, 0), 5: (0, 1)}
  for r in (1, 2, 7, 6):
    coef[r] = (1, -1j * _SIN1)
  for r in (9, 8, 3, 4):
    coef[r] = (1, 1j * _SIN1)
  primary = {1: 1, 2: 2, 3: 7, 4: 6}
  d2 = np.arange(64)
  col = lambda c: 16 * (d2 // 8) + 8 * c + d2 % 8
  fwd = np.zeros((5, 144, 128))
  inv = np.zeros((5, 128, 128))
  norm = 1.0 / (S * D)
  for g, res in enumerate(_GROUP_RES):
    for ri, rho in enumerate(res):
      al, be = coef[rho]
      for j in range(32):
        kd = rho + 10 * j
        row = 64 * ri + 16 * (j // 8) + j % 8
        w = np.exp(-2j * np.pi * ((d2 * kd) % D) / D)
        fwd[g, row, col(0)] = (al * w).real
        fwd[g, row + 8, col(0)] = (al * w).imag
        fwd[g, row, col(1)] = (be * w).real
        fwd[g, row + 8, col(1)] = (be * w).imag
        wi = np.conj(w)
        if g == 0:
          m = 1.0 if kd == 0 else 2.0
          inv[g, col(ri), row] = m * wi.real * norm
          inv[g, col(ri), row + 8] = m * (1j * wi).real * norm
        else:
          cr, ci = (wi, 1j * wi) if rho == primary[g] else (w, -1j * w)
          inv[g, col(0), row] = 2 * cr.real * norm
          inv[g, col(0), row + 8] = 2 * ci.real * norm
          inv[g, col(1), row] = 2 * _SIN1 * cr.imag * norm
          inv[g, col(1), row + 8] = 2 * _SIN1 * ci.imag * norm
  fwd[0, 128, col(0)] = (-1.0) ** d2
  inv[0, col(0), 8] = (-1.0) ** d2 * norm
  return fwd, inv


_FD, _GD = (np.asarray(m, np.float32).astype(jnp.bfloat16) for m in _d_matrices())


def _rdft5(u):
  s1, s2, d1, d2 = u[1] + u[4], u[2] + u[3], u[1] - u[4], u[2] - u[3]
  t = s1 + s2
  m1 = u[0] - 0.25 * t
  m2 = _C5 * (s1 - s2)
  return u[0] + t, m1 + m2, d1 + _RHO * d2, m1 - m2, _RHO * d1 - d2


def _irdft5(u0, p1, q1, p2, q2):
  p = p1 + p2
  m1 = u0 - 0.25 * p
  m2 = _C5 * (p1 - p2)
  a1, a2 = m1 + m2, m1 - m2
  b1, b2 = q1 + _RHO * q2, _RHO * q1 - q2
  return [u0 + p, a1 - b1, a2 - b2, a2 + b2, a1 + b1]


def _dft4(z):
  (ar, ai), (br, bi), (cr, ci), (dr, di) = z
  pr, pi, qr, qi = ar + cr, ai + ci, ar - cr, ai - ci
  rr, ri, sr, si = br + dr, bi + di, br - dr, bi - di
  return [(pr + rr, pi + ri), (qr + si, qi - sr), (pr - rr, pi - ri), (qr - si, qi + sr)]


def _dft4_output(z, c):
  (ar, ai), (br, bi), (cr, ci), (dr, di) = z
  if c % 2 == 0:
    pr, pi, qr, qi = ar + cr, ai + ci, br + dr, bi + di
    return (pr + qr, pi + qi) if c == 0 else (pr - qr, pi - qi)
  pr, pi, qr, qi = ar - cr, ai - ci, br - dr, bi - di
  return (pr + qi, pi - qr) if c == 1 else (pr - qi, pi + qr)


def _twiddle16(z, e):
  r, i = z
  if e == 0:
    return z
  if e == 4:
    return i, -r
  if e == 2:
    return (r + i) * _R2, (i - r) * _R2
  if e == 6:
    return (i - r) * _R2, (r + i) * (-_R2)
  c, s = {1: (_C8, _S8), 3: (_S8, _C8), 9: (-_C8, -_S8)}[e]
  return r * c + i * s, i * c - r * s


def _swap(z):
  return [(i, r) for r, i in z]


def _cmul(a, b):
  return a[0] * b[0] - a[1] * b[1], a[0] * b[1] + a[1] * b[0]


def _root(k):
  angle = (k % S).astype(f32) * (2 * np.pi / S)
  return jnp.cos(angle), -jnp.sin(angle)


def _strassen_left(a11, a12, a21, a22):
  return a11 + a22, a21 + a22, a11, a22, a11 + a12, a21 - a11, a12 - a22


def _strassen_right(b11, b12, b21, b22):
  return b11 + b22, b11, b12 - b22, b21 - b11, b22, b11 + b12, b21 + b22


def _strassen_result(m):
  return m[0] + m[3] - m[4] + m[6], m[2] + m[4], m[1] + m[3], m[0] - m[1] + m[2] + m[5]


def _tree_sum(parts):
  while len(parts) > 1:
    parts = [parts[i] + parts[i + 1] if i + 1 < len(parts) else parts[i]
             for i in range(0, len(parts), 2)]
  return parts[0]


def _kernel(x_hbm, wr_hbm, wi_hbm, w1t_hbm, b1_hbm, w2_hbm, b2_hbm, c_hbm, wmod_hbm,
            fd_hbm, gd_hbm, out_hbm,
            x_v, wr_v, wi_v, w1t_v, b1_v, w2_v, b2_v, c_v, wmod_v, fd_v, gd_v, fs_v,
            modb, actb, b1b, b2b, xt0, xt1, rhs0, rhs1, shift_v, z_v, t_v, wsh, x1_v, mean_v, h_v, h5_v, u_v, at_v, d_v, o_v,
            in_sem, out_sem):
  xt, rhs_v = (xt0, xt1), (rhs0, rhs1)
  copies = {}

  def fetch(name, pairs):
    sem = in_sem.at[len(copies)]
    copies[name] = [pltpu.make_async_copy(src, dst, sem) for src, dst in pairs]
    for cp in copies[name]:
      cp.start()

  def wait(*names):
    for name in names:
      for cp in copies[name]:
        cp.wait()

  def lanes(j):
    return slice(128 * j, 128 * j + 128)

  def tile_rows(t):
    return pl.ds(pl.multiple_of(t * 128, 128), 128)

  def x_pairs(i):
    return [(x_hbm.at[0, tile_rows(2 * i + a), :], x_v.at[2 * i + a]) for a in range(2)]

  def fetch_mod(m):
    fetch(f"m{m}", [(wmod_hbm.at[:, lanes(j)], wmod_v.at[j]) for j in range(ND * m, ND * m + ND)])

  fetch("c", [(c_hbm, c_v)])
  fetch("b1", [(b1_hbm, b1_v)])
  fetch("b2", [(b2_hbm, b2_v)])
  fetch_mod(1)
  for i in range(NT // 2):
    for src, dst in x_pairs(i):
      pltpu.make_async_copy(src, dst, in_sem.at[X_SEM + i]).start()
    if i == 0:
      fetch("fd", [(fd_hbm, fd_v)])
  fetch_mod(0)
  for jb in range(4):
    rows = slice(80 * jb, 80 * jb + 80 if jb < 3 else KD)
    fetch(f"w{jb}", [(wr_hbm.at[rows], wr_v.at[rows]), (wi_hbm.at[rows], wi_v.at[rows])])
  fetch("gd", [(gd_hbm, gd_v)])
  for m in (2, 3, 4):
    fetch_mod(m)
  fetch("w1t", [(w1t_hbm, w1t_v)])
  fetch("w2m", [(w2_hbm, w2_v)])
  fetch_mod(5)

  def wait_x(i):
    for src, dst in x_pairs(i):
      pltpu.make_async_copy(src, dst, in_sem.at[X_SEM + i]).wait()

  wait("c", "b1", "b2")
  sub = lax.broadcasted_iota(jnp.int32, (8, 128), 0)
  lane = lax.broadcasted_iota(jnp.int32, (8, 128), 1)
  freq = 128 * (lane % 16) + 16 * (lane // 16)
  base, base_step = _root(sub * freq), _root(8 * freq)
  turn, turn_step = _root(sub), _root(jnp.full((8, 128), 8, jnp.int32))
  for r in range(0, 128, 16):
    pair = []
    for _ in range(2):
      pair.append((base, turn))
      base, turn = _cmul(base, base_step), _cmul(turn, turn_step)
    cur = [b for b, _ in pair]
    for k1 in range(16):
      for part in range(2):
        rows16 = jnp.concatenate([v[part] for v in cur], axis=0)
        rows16 = pltpu.roll(rows16, k1, 1) if k1 else rows16
        fs_v[k1, part, r:r + 16, :] = rows16.astype(bf16)
      cur = [_cmul(v, s) for v, (_, s) in zip(cur, pair)]

  ri = lax.broadcasted_iota(jnp.int32, (144, 128), 0)
  ci = lax.broadcasted_iota(jnp.int32, (144, 128), 1)
  eye_ones = jnp.where((ri == ci) | (ri >= 128), 1.0, 0.0).astype(bf16)
  eye = eye_ones[0:128]

  def to_columns(row, dst):
    n, marks = row.shape[1], []
    for j in range(0, n, 128):
      w = min(128, n - j)
      tile = jnp.broadcast_to(row[:, j:j + w], (128, w))
      col = lax.dot_general(eye[:w, :w], tile, _NT_DIMS, preferred_element_type=f32)
      dst[j:j + w, :] = col
      marks.append(col[0:8])
    return marks

  cf = c_v[...].astype(f32)
  act = jnp.broadcast_to((cf * jax.nn.sigmoid(cf)).astype(bf16), (16, D))
  to_columns(act[0:1], actb)
  to_columns(b1_v[...].reshape(1, F), b1b)
  to_columns(b2_v[...].reshape(1, D), b2b)

  def modulation(m):
    w = jnp.concatenate([wmod_v[j] for j in range(ND * m, ND * m + ND)], axis=1)
    row = jnp.dot(act, w, preferred_element_type=f32)[0:1, :].astype(bf16)
    return (1.0 + row.astype(f32)).astype(bf16) if m in (1, 4) else row

  wait("m1")
  to_columns(modulation(1), modb.at[1])
  wait_x(0)
  wait("fd")
  zero = fd_v[0, 128:144, :].astype(f32).astype(jnp.int32)[1, 0]

  def after(value, other):
    return value if other is None else jnp.where(zero == 0, value, other)

  def transpose_tiles(k, p):
    total, marks = None, []
    for j in range(ND):
      xj = jnp.concatenate([x_v[4 * k + 2 * p + a, :, lanes(j)] for a in range(2)], axis=0)
      res = lax.dot_general(eye_ones, xj, _NT_DIMS, preferred_element_type=f32)
      for a in range(2):
        xt[p][k, a, lanes(j), :] = res[0:128, lanes(a)]
      total = res[128:136] if total is None else total + res[128:136]
      marks += [res[r:r + 8, 0:128] for r in (0, 64)]
    return [total[:, lanes(a)] * (1.0 / D) for a in range(2)], marks

  def radix10(dst, load):
    for r8 in range(8):
      v = load([slice(64 * d1 + 8 * r8, 64 * d1 + 8 * r8 + 8) for d1 in range(10)])
      e0, e1r, e1i, e2r, e2i = _rdft5([v[2 * b] + v[(5 + 2 * b) % 10] for b in range(5)])
      o0, o1r, o1i, o2r, o2i = _rdft5([v[2 * b] - v[(5 + 2 * b) % 10] for b in range(5)])
      for g, pair in enumerate(((e0, o0), (o1r, o1i), (e2r, e2i), (o2r, o2i), (e1r, e1i))):
        dst[g, 16 * r8:16 * r8 + 16, :] = jnp.concatenate(pair, axis=0).astype(bf16)

  def length64(srcs, scales, dsts):
    marks = []
    for g in range(5):
      rhs = jnp.concatenate([src[g + zero] for src in srcs], axis=1)
      res = jnp.dot(fd_v[g, 0:144 if g == 0 else 128, :], rhs, preferred_element_type=f32)
      marks += [res[r:r + 8, 0:128] for r in (0, 64)]
      rows = [(10 * jb + rho, 64 * k + 16 * jb)
              for k, rho in enumerate(_GROUP_RES[g]) for jb in range(4)]
      for q, r0 in rows + ([(40, 128)] if g == 0 else []):
        for a, (scale, dst) in enumerate(zip(scales, dsts)):
          for h in (0, 8):
            dst[16 * q + h:16 * q + h + 8, :] = res[r0 + h:r0 + h + 8, lanes(a)] * scale
    return marks

  def first_stage(k, p, means, marks=()):
    rstds, marks = [], iter(marks)
    for a in range(2):
      squares = []

      def load(slices):
        mean = after(means[a], next(marks, None))
        xc = [xt[p][k, a, rows, :] - mean for rows in slices]
        squares.append(_tree_sum([v * v for v in xc]))
        return [v * modb[1, rows, :] for v, rows in zip(xc, slices)]

      radix10(rhs_v[p].at[a], load)
      var = jnp.sum(_tree_sum(squares), axis=0, keepdims=True) * (1.0 / D)
      rstds.append(jnp.broadcast_to(lax.rsqrt(var + EPS), (8, 128)))
    return rstds

  def second_stage(k, p, rstds):
    return length64([rhs_v[p].at[a] for a in range(2)], rstds,
                    [z_v.at[4 * k + 2 * p + a] for a in range(2)])

  def phase1(k, carry):
    rstds, means = carry
    for p in range(2):
      wait_x(2 * k + p + 2)
      marks = second_stage(k, p, rstds)
      ahead, more = transpose_tiles(k + 1, p)
      rstds, means = first_stage(k + p, 1 - p, means, [None] * 2 + marks + more), ahead
    return rstds, means

  with jax.named_scope("phase1"):
    means, _ = transpose_tiles(0, 0)
    wait_x(1)
    ahead, marks = transpose_tiles(0, 1)
    rstds, means = lax.fori_loop(0, 3, phase1, (first_stage(zero, 0, means, [None] * 6 + marks), ahead))
    marks = second_stage(3, 0, rstds)
    second_stage(3, 1, first_stage(3, 1, means, [None] * 6 + marks))

  shift_masks = [((lane >> i) & 1) == 1 for i in range(4)]

  def shuffle_filter(m, pin=None):
    pin = None if pin is None else pltpu.bitcast(pin, u32)
    for a, w_v in enumerate((wr_v, wi_v)):
      cur = [None] * 16
      for t in range(16):
        if m < 20:
          word = pltpu.bitcast(w_v[16 * m:16 * m + 16, lanes(t)], u32)
        else:
          word = pltpu.bitcast(jnp.broadcast_to(w_v[KD - 1:KD, lanes(t)].astype(f32), (8, 128)), u32)
        cur[(-t) % 16] = pltpu.roll(word, t, 1) if t else after(word, pin)
      for i in range(4):
        cur = [jnp.where(shift_masks[i], cur[(j - (1 << i)) % 16], cur[j]) for j in range(16)]
      for k1 in range(16):
        wsh[a, k1, 8 * m:8 * m + 8, :] = cur[k1]

  def filter_rows(a, k1, jb):
    rows = []
    for i in range(5):
      word = wsh[a, k1, pl.ds(40 * jb + i, 8, stride=5), :]
      rows.append(pltpu.bitcast(word << 16, f32))
      rows.append(pltpu.bitcast(word & np.uint32(0xFFFF0000), f32))
    if jb == 3:
      rows.append(pltpu.bitcast(wsh[a, k1, 160:168, :], f32))
    return jnp.stack(rows, axis=0)

  def modulation_tile(j, pin):
    sums = []
    for r0 in range(0, D, 64):
      w = wmod_v[j, r0:r0 + 64, :].astype(f32)
      terms = [w[r:r + 8] * actb[r0 + r:r0 + r + 8, :] for r in range(0, 64, 8)]
      terms[0] = after(terms[0], pin)
      sums.append(_tree_sum(terms))
    row = jnp.sum(_tree_sum(sums), axis=0, keepdims=True).astype(bf16)
    return (1.0 + row.astype(f32)).astype(bf16) if j // ND == 4 else row

  def spectral(jb, c):
    n = 11 if jb == 3 else 10
    rows = slice(160 * jb, 160 * jb + 16 * n)

    def load(t):
      z = z_v[t, rows, :].reshape(n, 16, 128)
      return z[:, 0:8], z[:, 8:16]

    inner = [_twiddle16(_dft4_output([load(4 * a + b) for a in range(4)], c), b * c)
             for b in range(4)]
    back, marks = [], []
    for e, (ar, ai) in enumerate(_dft4(inner)):
      k1 = c + 4 * e
      fr, fi = fs_v[k1, 0], fs_v[k1, 1]
      lhs = jnp.concatenate([ar, ai], axis=1).reshape(16 * n, 128).astype(bf16)
      p = jnp.dot(lhs, jnp.concatenate([fr, fi], axis=1), preferred_element_type=f32)
      marks.append(p[0:8, 0:128])
      p = p.reshape(n, 16, 256)
      x = (p[:, 0:8, 0:128] - p[:, 8:16, 128:256], p[:, 0:8, 128:256] + p[:, 8:16, 0:128])
      if k1 == 0:
        shift = shift_v[rows, :].reshape(n, 16, 128)
        x = (x[0] + shift[:, 0:8], x[1] + shift[:, 8:16])
      y = jnp.concatenate(_cmul(x, (filter_rows(0, k1, jb), filter_rows(1, k1, jb))), axis=1)
      y = y.reshape(16 * n, 128).astype(bf16)
      p = lax.dot_general(y, jnp.concatenate([fr, fi], axis=0), _NT_DIMS,
                          preferred_element_type=f32)
      p = p.reshape(n, 16, 256)
      back.append((p[:, 0:8, 0:128] + p[:, 8:16, 128:256],
                   p[:, 8:16, 0:128] - p[:, 0:8, 128:256]))
    for b, (tr, ti) in enumerate(_swap([_twiddle16(v, b * c)
                                        for b, v in enumerate(_dft4(_swap(back)))])):
      t_v[b, c, rows, :] = jnp.concatenate([tr, ti], axis=1).reshape(16 * n, 128)
    return marks

  with jax.named_scope("phase2"):
    wait("m0", "w0", "w1")
    shuffle_filter(0)
    marks = to_columns(modulation(0), modb.at[0])
    shuffle_filter(1, marks[0])
    shuffle_filter(2, marks[4])
    radix10(rhs_v[0].at[0], lambda slices: [modb[zero, rows, :] for rows in slices])
    marks = length64([rhs_v[0].at[0]], [jnp.where(lane == 0, float(S), 0.0)], [shift_v])
    shuffle_filter(3, marks[0])
    shuffle_filter(4, marks[6])
    ready = []
    for jb in range(4):
      if jb == 1:
        wait("w2", "w3")
      elif jb == 3:
        wait("gd", "m2", "m3", "m4")
      todo = list(range(5 * jb + 5, 5 * jb + 10 + (jb == 2))) if jb < 3 else []
      for c in range(4):
        marks = spectral(jb, c)
        for m, mark in zip(todo[c::4], marks[0::2]):
          shuffle_filter(m, mark)
        if jb == 3:
          for j, row in ready:
            to_columns(row, modb.at[j // ND, lanes(j % ND)])
          ready = [(j, modulation_tile(j, mark))
                   for j, mark in zip(range(2 * ND + 4 * c, 5 * ND), marks)]

  def inverse_d(b, g):
    def last_radix4(q):
      z = [(t_v[b, c, 16 * q:16 * q + 8, :], t_v[b, c, 16 * q + 8:16 * q + 16, :])
           for c in range(4)]
      return _swap(_dft4(_swap(z)))

    blocks = []
    for rho in _GROUP_RES[g]:
      for jb in range(4):
        z = last_radix4(10 * jb + rho)
        if rho == 0 and jb == 0:
          z = [(r, jnp.where(sub == 0, nq[0], i)) for (r, i), nq in zip(z, last_radix4(40))]
        blocks.append(jnp.concatenate([jnp.concatenate(p, axis=0) for p in z], axis=1))
    rhs = jnp.concatenate(blocks, axis=0).astype(bf16)
    y = jnp.dot(gd_v[g], rhs, preferred_element_type=f32)
    for a in range(TPC):
      z_v[4 * a + b, lanes(g), :] = y[:, lanes(a)]
    return y

  def residual(p, odd):
    b = 2 * p + odd
    pin = yield
    for a in range(TPC):
      t = 4 * a + b
      sums = []
      for r8 in range(8):
        ab = [(z_v[t, 128 * g + 16 * r8:128 * g + 16 * r8 + 8, :],
               z_v[t, 128 * g + 16 * r8 + 8:128 * g + 16 * r8 + 16, :]) for g in range(5)]
        ev = _irdft5(after(ab[0][0], pin), ab[4][0], ab[4][1], ab[2][0], ab[2][1])
        od = _irdft5(ab[0][1], ab[1][0], ab[1][1], ab[3][0], ab[3][1])
        part = []
        for k in range(5):
          for d1, y in ((2 * k, ev[k] + od[k]), ((5 + 2 * k) % 10, ev[k] - od[k])):
            rows = slice(64 * d1 + 8 * r8, 64 * d1 + 8 * r8 + 8)
            x1 = xt[p][a, odd, rows, :] + modb[2, rows, :] * y
            x1_v[t, rows, :] = x1
            part.append(x1)
        sums.append(_tree_sum(part))
        if r8 == 7:
          mean = jnp.sum(_tree_sum(sums), axis=0, keepdims=True) * (1.0 / D)
          mean_v[t] = jnp.broadcast_to(mean, (8, 128))
        pin = yield

  def inverse_std(t, mean):
    sums = []
    for r0 in range(0, D // 8, 8):
      xc = [x1_v[t + zero, 8 * r:8 * r + 8, :] - mean for r in range(r0, r0 + 8)]
      sums.append(_tree_sum([v * v for v in xc]))
    var = jnp.sum(_tree_sum(sums), axis=0, keepdims=True) * (1.0 / D)
    return jnp.broadcast_to(lax.rsqrt(var + EPS), (8, 128))

  def normalize(b):
    pin = yield
    for p in range(2):
      tiles = [4 * a + b for a in (p, p + 2)]
      means, rstds = [], []
      for t in tiles:
        means.append(after(mean_v[t + zero], pin))
        rstds.append(inverse_std(t, means[-1]))
        pin = yield

      def rows16(k, r, scale):
        h = [(x1_v[tiles[k] + zero, rows, :] - means[k]) * scale * modb[4, rows, :] + modb[3, rows, :]
             for rows in (slice(r, r + 8), slice(r + 8, r + 16))]
        return jnp.concatenate(h, axis=0)

      for r0 in range(0, 256, 64):
        s0, s1 = after(rstds[0], pin), after(rstds[1], pin)
        for r in range(r0, r0 + 64, 16):
          quads = rows16(0, r, s0), rows16(1, r, s1), rows16(0, 256 + r, s0), rows16(1, 256 + r, s1)
          for i, v in enumerate(_strassen_right(*quads)):
            h_v[i, p, r:r + 16, :] = v.astype(bf16)
        pin = yield
      for k in range(2):
        scale = after(rstds[k], pin)
        for r in range(0, 128, 16):
          h5_v[p + 2 * k, r:r + 16, :] = rows16(k, 512 + r, scale).astype(bf16)
      pin = yield

  def prepare_w2():
    pin = yield
    for k in range(KT):
      w = min(128, FH - 128 * k)
      for j in range(ND):
        flipped = []
        for half in range(2):
          blk = w2_v[FH * half + 128 * k:FH * half + 128 * k + w, lanes(j)].astype(f32)
          flipped.append(jnp.concatenate([after(blk[0:8], pin), blk[8:]], axis=0).T)
        quads = flipped[0][0:64], flipped[1][0:64], flipped[0][64:128], flipped[1][64:128]
        for i, v in enumerate(_strassen_left(*quads)):
          d_v[i, k, 64 * j:64 * j + 64, 0:w] = v.astype(bf16)
        pin = yield

  def start(side):
    next(side)
    return side

  def step(side, value, pieces=1):
    for _ in range(pieces):
      try:
        side.send(value)
      except StopIteration:
        return

  def finish(side):
    for _ in side:
      pass

  class Paced:
    def __init__(self, *tasks):
      self.tasks, self.count = tasks, 0

    def __call__(self, result):
      for every, task in self.tasks:
        if self.count % every == 0:
          task(result[0:8, 0:128])
      self.count += 1
      return result

  def mlp_up(lo, hi, tick, block=UP_ROWS, prepare=False):
    right = [jnp.concatenate([h_v[i + zero, p] for p in range(2)], axis=1) for i in range(7)]
    right5 = jnp.concatenate([h5_v[a + zero] for a in range(TPC)], axis=1)
    for r0 in range(lo, hi, block):
      top, bottom = slice(r0, r0 + block), slice(FH + r0, FH + r0 + block)
      if prepare:
        quads = [w1t_v[rows, c:c + 256].astype(f32) for rows in (top, bottom) for c in (0, 256)]
        left = [v.astype(bf16) for v in _strassen_left(*quads)]
        for i, v in enumerate(left):
          for k in range(2):
            u_v[i, k, top, :] = v[:, lanes(k)]
      else:
        left = [jnp.concatenate([u_v[i, k, top, :] for k in range(2)], axis=1) for i in range(7)]
      extra = [tick(jnp.dot(w1t_v[rows, 512:D], right5, preferred_element_type=f32))
               for rows in (top, bottom)]
      c = _strassen_result([tick(jnp.dot(a, b, preferred_element_type=f32))
                            for a, b in zip(left, right)])
      acts = []
      for q in range(4):
        rows = (top, bottom)[q // 2]
        u = c[q] + extra[q // 2][:, 256 * (q % 2):256 * (q % 2) + 256]
        r = jnp.maximum(u + jnp.concatenate([b1b[rows, :]] * 2, axis=1), 0.0)
        acts.append(r * r)
      for i, v in enumerate(_strassen_right(*acts)):
        for p in range(2):
          at_v[i, p, top, :] = v[:, lanes(p)].astype(bf16)

  def out_copy(t, cols, sem):
    return pltpu.make_async_copy(o_v.at[tile_rows(t), cols], out_hbm.at[0, tile_rows(t), cols],
                                 out_sem.at[sem])

  def mlp_down(b, tick, done=None):
    right = [jnp.concatenate([at_v[i, p] for p in range(2)], axis=1) for i in range(7)]
    for j in range(ND):
      halves = [[] for _ in range(4)]
      for r0 in range(0, 64, DOWN_ROWS):
        rows = slice(64 * j + r0, 64 * j + r0 + DOWN_ROWS)
        left = [jnp.concatenate([d_v[i, k, rows, 0:min(128, FH - 128 * k)] for k in range(KT)],
                                axis=1) for i in range(7)]
        c = _strassen_result([tick(jnp.dot(a, b_, preferred_element_type=f32))
                              for a, b_ in zip(left, right)])
        for q in range(4):
          feat = 128 * j + 64 * (q // 2) + r0
          feat = slice(feat, feat + DOWN_ROWS)
          halves[q].append([
              (x1_v[4 * (2 * (q % 2) + p) + b, feat, :] +
               modb[5, feat, :] * (c[q][:, lanes(p)] + b2b[feat, :])).astype(bf16)
              for p in range(2)])
      for a in range(TPC):
        res = jnp.concatenate([part[a % 2] for q in (a // 2, 2 + a // 2) for part in halves[q]],
                              axis=0)
        o_v[tile_rows(4 * a + b), lanes(j)] = res.T
      if done:
        done(j)

  with jax.named_scope("phase3_head"):
    for g in range(5):
      inverse_d(0, g)
      if g == 1:
        for j, row in ready:
          to_columns(row, modb.at[j // ND, lanes(j % ND)])
    res, norm = start(residual(0, zero)), start(normalize(zero))
    step(res, None, 0)
    count = 0
    for b in range(1, NCH):
      for g in range(5):
        y = inverse_d(b, g)
        for r in range(0, 128, 40):
          step(res if count < 32 else norm, y[r:r + 8, 0:128], 1 if count < 32 else 1)
          count += 1
    finish(res)
    finish(norm)
    wait("w1t")
    res = start(residual(0, zero + 1))
    piece = lambda side: functools.partial(step, side)
    mlp_up(0, 192, Paced((2, piece(res))), 32, prepare=True)
    wait("w2m", "m5")
    flip = start(prepare_w2())
    to_columns(modulation(5), modb.at[5])
    mlp_up(192, FH, Paced((30, piece(res)), (5, piece(flip))), 32, prepare=True)
    finish(flip)
    finish(res)

  def chunk(b, carry):
    norm = start(normalize(b + 1))
    step(norm, None)
    mlp_down(b, Paced((DOWN_PACE, piece(norm))))
    finish(norm)
    res = start(residual(1, jnp.minimum(b, 1)))
    mlp_up(0, FH, Paced((UP_PACE, piece(res))))
    finish(res)
    for a in range(TPC):
      out_copy(4 * a + b, slice(None), 4 * a + b).start()
    return carry

  with jax.named_scope("phase3_loop"):
    lax.fori_loop(0, NCH - 1, chunk, 0)

  with jax.named_scope("phase3_tail"):
    last = NCH - 1
    early, late = slice(0, 128 * (ND - 1)), slice(128 * (ND - 1), D)

    def send_early(j):
      if j == ND - 2:
        for a in range(TPC):
          out_copy(4 * a + last, early, 4 * a + last).start()

    mlp_down(last, Paced(), done=send_early)
    for a in range(TPC):
      out_copy(4 * a + last, late, NT + a).start()
    for t in range(NT):
      out_copy(t, early if t % 4 == last else slice(None), t).wait()
    for a in range(TPC):
      out_copy(4 * a + last, late, NT + a).wait()


@jax.jit
def pallas_adaLN_cond__spectral_gfnet__dense_activation_squared_relu__prompt_kernel(
    A_x: jax.Array,
    A_w_r: jax.Array,
    A_w_i: jax.Array,
    B_x: jax.Array,
    B_w1: jax.Array,
    B_b1: jax.Array,
    B_w2: jax.Array,
    B_b2: jax.Array,
    c: jax.Array,
    w_mod: jax.Array,
):
  del B_x
  vmem = pltpu.VMEM
  operands = (A_x, A_w_r.T, A_w_i.T, B_w1.T, B_b1, B_w2, B_b2, c, w_mod, _FD, _GD)
  scratch = [
      vmem((NT, 128, D), bf16), vmem((KD, S), bf16), vmem((KD, S), bf16),
      vmem((F, D), bf16), vmem((F,), bf16), vmem((F, D), bf16), vmem((D,), bf16),
      vmem((1, D), bf16), vmem((6 * ND, D, 128), bf16),
      vmem((5, 144, 128), bf16), vmem((5, 128, 128), bf16), vmem((16, 2, 128, 128), bf16),
      vmem((6, D, 128), f32), vmem((D, 128), f32), vmem((F, 128), f32), vmem((D, 128), f32),
      vmem((4, 2, D, 128), f32), vmem((4, 2, D, 128), f32),
      vmem((2, 5, 128, 128), bf16), vmem((2, 5, 128, 128), bf16),
      vmem((656, 128), f32),
      vmem((NT, 656, 128), f32),
      vmem((4, 4, 656, 128), f32),
      vmem((2, 16, 168, 128), u32),
      vmem((NT, D, 128), f32),
      vmem((NT, 8, 128), f32),
      vmem((7, 2, 256, 128), bf16), vmem((TPC, 128, 128), bf16),
      vmem((7, 2, FH, 128), bf16),
      vmem((7, 2, FH, 128), bf16),
      vmem((7, KT, D // 2, 128), bf16),
      vmem((S, D), bf16),
      pltpu.SemaphoreType.DMA((X_SEM + NT // 2,)), pltpu.SemaphoreType.DMA((NT + TPC,)),
  ]
  return pl.pallas_call(
      _kernel,
      out_shape=jax.ShapeDtypeStruct(A_x.shape, A_x.dtype),
      in_specs=[pl.BlockSpec(memory_space=pl.ANY)] * len(operands),
      out_specs=pl.BlockSpec(memory_space=pl.ANY),
      scratch_shapes=scratch,
      compiler_params=pltpu.CompilerParams(vmem_limit_bytes=100 * 2**20),
      name="adaln_gfnet_mlp",
  )(*operands)
```

```python
import functools

import numpy as np

import jax
import jax.numpy as jnp
from jax import lax
import jax.experimental.pallas as pl
import jax.experimental.pallas.tpu as pltpu

S, D, F = 2048, 640, 1728
KD = D // 2 + 1
NT = S // 128
ND = D // 128
EPS = 1e-5
TPC = 4
NCH = NT // TPC
FH = F // 2
KT = -(-FH // 128)
UP_BLOCKS = (112,) * 7 + (48, 32)
DOWN_BLOCKS = ((0, 1), (2, 3), (4,))

bf16, f32, u32 = jnp.bfloat16, jnp.float32, jnp.uint32
_NT_DIMS = (((1,), (1,)), ((), ()))

_SIN1, _SIN2 = np.sin(2 * np.pi / 5), np.sin(4 * np.pi / 5)
_RHO = float(_SIN2 / _SIN1)
_C5 = float(np.sqrt(5.0) / 4)
_R2 = float(np.sqrt(0.5))
_C8, _S8 = float(np.cos(np.pi / 8)), float(np.sin(np.pi / 8))
_GROUP_RES = ((0, 5), (1, 9), (2, 8), (3, 7), (4, 6))


def _d_matrices():
  coef = {0: (1, 0), 5: (0, 1)}
  for r in (1, 2, 7, 6):
    coef[r] = (1, -1j * _SIN1)
  for r in (9, 8, 3, 4):
    coef[r] = (1, 1j * _SIN1)
  primary = {1: 1, 2: 2, 3: 7, 4: 6}
  d2 = np.arange(64)
  col = lambda c: 16 * (d2 // 8) + 8 * c + d2 % 8
  fwd = np.zeros((5, 144, 128))
  inv = np.zeros((5, 128, 128))
  norm = 1.0 / (S * D)
  for g, res in enumerate(_GROUP_RES):
    for k, rho in enumerate(res):
      al, be = coef[rho]
      for j in range(32):
        kd = rho + 10 * j
        row = 64 * k + 16 * (j // 8) + j % 8
        w = np.exp(-2j * np.pi * ((d2 * kd) % D) / D)
        fwd[g, row, col(0)] = (al * w).real
        fwd[g, row + 8, col(0)] = (al * w).imag
        fwd[g, row, col(1)] = (be * w).real
        fwd[g, row + 8, col(1)] = (be * w).imag
        wi = np.conj(w)
        if g == 0:
          m = 1.0 if kd == 0 else 2.0
          inv[g, col(k), row] = m * wi.real * norm
          inv[g, col(k), row + 8] = m * (1j * wi).real * norm
        else:
          cr, ci = (wi, 1j * wi) if rho == primary[g] else (w, -1j * w)
          inv[g, col(0), row] = 2 * cr.real * norm
          inv[g, col(0), row + 8] = 2 * ci.real * norm
          inv[g, col(1), row] = 2 * _SIN1 * cr.imag * norm
          inv[g, col(1), row + 8] = 2 * _SIN1 * ci.imag * norm
  fwd[0, 128, col(0)] = (-1.0) ** d2
  inv[0, col(0), 8] = (-1.0) ** d2 * norm
  return fwd, inv


_FD, _GD = (np.asarray(m, np.float32).astype(jnp.bfloat16) for m in _d_matrices())


def _rdft5(u):
  s1, s2, d1, d2 = u[1] + u[4], u[2] + u[3], u[1] - u[4], u[2] - u[3]
  t = s1 + s2
  m1 = u[0] - 0.25 * t
  m2 = _C5 * (s1 - s2)
  return u[0] + t, m1 + m2, d1 + _RHO * d2, m1 - m2, _RHO * d1 - d2


def _irdft5(u0, p1, q1, p2, q2):
  p = p1 + p2
  m1 = u0 - 0.25 * p
  m2 = _C5 * (p1 - p2)
  a1, a2 = m1 + m2, m1 - m2
  b1, b2 = q1 + _RHO * q2, _RHO * q1 - q2
  return [u0 + p, a1 - b1, a2 - b2, a2 + b2, a1 + b1]


def _dft4(z):
  (ar, ai), (br, bi), (cr, ci), (dr, di) = z
  pr, pi, qr, qi = ar + cr, ai + ci, ar - cr, ai - ci
  rr, ri, sr, si = br + dr, bi + di, br - dr, bi - di
  return [(pr + rr, pi + ri), (qr + si, qi - sr), (pr - rr, pi - ri), (qr - si, qi + sr)]


def _dft4_output(z, c):
  (ar, ai), (br, bi), (cr, ci), (dr, di) = z
  if c % 2 == 0:
    pr, pi, qr, qi = ar + cr, ai + ci, br + dr, bi + di
    return (pr + qr, pi + qi) if c == 0 else (pr - qr, pi - qi)
  pr, pi, qr, qi = ar - cr, ai - ci, br - dr, bi - di
  return (pr + qi, pi - qr) if c == 1 else (pr - qi, pi + qr)


def _twiddle16(z, e):
  r, i = z
  if e == 0:
    return z
  if e == 4:
    return i, -r
  if e == 2:
    return (r + i) * _R2, (i - r) * _R2
  if e == 6:
    return (i - r) * _R2, (r + i) * (-_R2)
  c, s = {1: (_C8, _S8), 3: (_S8, _C8), 9: (-_C8, -_S8)}[e]
  return r * c + i * s, i * c - r * s


def _swap(z):
  return [(i, r) for r, i in z]


def _cmul(a, b):
  return a[0] * b[0] - a[1] * b[1], a[0] * b[1] + a[1] * b[0]


def _root(k):
  angle = (k % S).astype(f32) * (2 * np.pi / S)
  return jnp.cos(angle), -jnp.sin(angle)


def _strassen_left(a11, a12, a21, a22):
  return a11 + a22, a21 + a22, a11, a22, a11 + a12, a21 - a11, a12 - a22


def _strassen_right(b11, b12, b21, b22):
  return b11 + b22, b11, b12 - b22, b21 - b11, b22, b11 + b12, b21 + b22


def _strassen_result(m):
  return m[0] + m[3] - m[4] + m[6], m[2] + m[4], m[1] + m[3], m[0] - m[1] + m[2] + m[5]


def _tree_sum(parts):
  while len(parts) > 1:
    parts = [parts[i] + parts[i + 1] if i + 1 < len(parts) else parts[i]
             for i in range(0, len(parts), 2)]
  return parts[0]


def _lanes(j):
  return slice(128 * j, 128 * j + 128)


def _tile_rows(t):
  return pl.ds(pl.multiple_of(t * 128, 128), 128)


def _begin(side):
  next(side)
  return side


def _step(side, value):
  try:
    return side.send(value)
  except StopIteration:
    return None


def _finish(side):
  for _ in side:
    pass


class _Paced:
  def __init__(self, *tasks):
    self.tasks, self.count = tasks, 0

  def __call__(self, result):
    for every, task in self.tasks:
      if self.count % every == 0:
        task(result[0:8, 0:128])
    self.count += 1
    return result


def _kernel(x_hbm, wr_hbm, wi_hbm, w1t_hbm, b1_hbm, w2_hbm, b2_hbm, c_hbm, wmod_hbm,
            fd_hbm, gd_hbm, out_hbm,
            x_v, wr_v, wi_v, w1t_v, b1_v, w2_v, b2_v, c_v, wmod_v, fd_v, gd_v, fs_v,
            modb, actb, b1b, b2b, xt, rhs_v, shift_v, z_v, t_v, wsh, x1_v, mean_v,
            h_v, h5_v, u_v, at_v, d_v, o_v, in_sem, out_sem):
  groups = {}

  def fetch(name, pairs):
    groups[name] = [pltpu.make_async_copy(src, dst, in_sem.at[len(groups)]) for src, dst in pairs]
    for copy in groups[name]:
      copy.start()

  def wait(name):
    for copy in groups[name]:
      copy.wait()

  def x_tiles(*tiles):
    return [(x_hbm.at[0, _tile_rows(t), :], x_v.at[t]) for t in tiles]

  def mod_tiles(*vectors):
    return [(wmod_hbm.at[:, _lanes(j)], wmod_v.at[j])
            for m in vectors for j in range(ND * m, ND * m + ND)]

  def filter_part(lo, hi):
    return [(wr_hbm.at[lo:hi], wr_v.at[lo:hi]), (wi_hbm.at[lo:hi], wi_v.at[lo:hi])]

  fetch("vectors", [(c_hbm, c_v), (b1_hbm, b1_v), (b2_hbm, b2_v)])
  fetch("scale", mod_tiles(1))
  for i in range(4):
    fetch(f"x{i}", ([(fd_hbm, fd_v)] if i == 2 else []) + x_tiles(2 * i, 2 * i + 1))
  for i in (4, 6):
    fetch(f"x{i}", x_tiles(*range(2 * i, 2 * i + 4)))
  fetch("filter0", mod_tiles(0) + filter_part(0, 80))
  fetch("filter1", filter_part(80, 160))
  fetch("filter2", filter_part(160, KD))
  fetch("mod", [(gd_hbm, gd_v)] + mod_tiles(2, 3, 4))
  fetch("w1", [(w1t_hbm, w1t_v)])
  fetch("w2", [(w2_hbm, w2_v)] + mod_tiles(5))

  wait("vectors")
  sub = lax.broadcasted_iota(jnp.int32, (8, 128), 0)
  lane = lax.broadcasted_iota(jnp.int32, (8, 128), 1)
  freq = 128 * (lane % 16) + 16 * (lane // 16)
  base, base_step = _root(sub * freq), _root(8 * freq)
  turn, turn_step = _root(sub), _root(jnp.full((8, 128), 8, jnp.int32))
  for r in range(0, 128, 16):
    pair = []
    for _ in range(2):
      pair.append((base, turn))
      base, turn = _cmul(base, base_step), _cmul(turn, turn_step)
    cur = [b for b, _ in pair]
    for k1 in range(16):
      for part in range(2):
        rows16 = jnp.concatenate([v[part] for v in cur], axis=0)
        rows16 = pltpu.roll(rows16, k1, 1) if k1 else rows16
        fs_v[k1, part, r:r + 16, :] = rows16.astype(bf16)
      cur = [_cmul(v, s) for v, (_, s) in zip(cur, pair)]

  ri = lax.broadcasted_iota(jnp.int32, (144, 128), 0)
  ci = lax.broadcasted_iota(jnp.int32, (144, 128), 1)
  eye_ones = jnp.where((ri == ci) | (ri >= 128), 1.0, 0.0).astype(bf16)
  eye = eye_ones[0:128]

  def to_columns(row, dst):
    n, marks = row.shape[1], []
    for j in range(0, n, 128):
      w = min(128, n - j)
      tile = jnp.broadcast_to(row[:, j:j + w], (128, w))
      col = lax.dot_general(eye[:w, :w], tile, _NT_DIMS, preferred_element_type=f32)
      dst[j:j + w, :] = col
      marks.append(col[0:8])
    return marks

  cf = c_v[...].astype(f32)
  n = (pltpu.bitcast(jnp.broadcast_to(cf[:, 0:128], (8, 128)), jnp.int32) >> 16) & 255
  always = ((n * (n + 1)) & 1) == 0

  def after(value, other):
    return value if other is None else jnp.where(always, value, other)

  act = jnp.broadcast_to((cf * jax.nn.sigmoid(cf)).astype(bf16), (16, D))
  to_columns(act[0:1], actb)
  to_columns(b1_v[...].reshape(1, F), b1b)
  to_columns(b2_v[...].reshape(1, D), b2b)

  def with_offset(row, m):
    row = row.astype(bf16)
    return (1.0 + row.astype(f32)).astype(bf16) if m in (1, 4) else row

  def modulation(m):
    w = jnp.concatenate([wmod_v[j] for j in range(ND * m, ND * m + ND)], axis=1)
    return with_offset(jnp.dot(act, w, preferred_element_type=f32)[0:1, :], m)

  def modulation_tile(j, pin):
    sums = []
    for r0 in range(0, D, 64):
      w = wmod_v[j, r0:r0 + 64, :].astype(f32)
      terms = [w[r:r + 8] * actb[r0 + r:r0 + r + 8, :] for r in range(0, 64, 8)]
      terms[0] = after(terms[0], pin)
      sums.append(_tree_sum(terms))
    return with_offset(jnp.sum(_tree_sum(sums), axis=0, keepdims=True), j // ND)

  wait("scale")
  to_columns(modulation(1), modb.at[1])

  def transpose_tiles(i):
    total, marks = None, []
    for j in range(ND):
      xj = jnp.concatenate([x_v[2 * i + a, :, _lanes(j)] for a in range(2)], axis=0)
      res = lax.dot_general(eye_ones, xj, _NT_DIMS, preferred_element_type=f32)
      for a in range(2):
        xt[2 * i + a, _lanes(j), :] = res[0:128, _lanes(a)]
      total = res[128:136] if total is None else total + res[128:136]
      marks += [res[r:r + 8, 0:128] for r in (0, 64)]
    return [total[:, _lanes(a)] * (1.0 / D) for a in range(2)], marks

  def radix10(dst, load):
    for r8 in range(8):
      v = load([slice(64 * d1 + 8 * r8, 64 * d1 + 8 * r8 + 8) for d1 in range(10)])
      e0, e1r, e1i, e2r, e2i = _rdft5([v[2 * b] + v[(5 + 2 * b) % 10] for b in range(5)])
      o0, o1r, o1i, o2r, o2i = _rdft5([v[2 * b] - v[(5 + 2 * b) % 10] for b in range(5)])
      for g, pair in enumerate(((e0, o0), (o1r, o1i), (e2r, e2i), (o2r, o2i), (e1r, e1i))):
        dst[g, 16 * r8:16 * r8 + 16, :] = jnp.concatenate(pair, axis=0).astype(bf16)

  def length64(srcs, scales, dsts):
    marks = []
    for g in range(5):
      rhs = jnp.concatenate([src[g] for src in srcs], axis=1)
      res = jnp.dot(fd_v[g, 0:144 if g == 0 else 128, :], rhs, preferred_element_type=f32)
      marks += [res[r:r + 8, 0:128] for r in (0, 64)]
      rows = [(10 * jb + rho, 64 * k + 16 * jb)
              for k, rho in enumerate(_GROUP_RES[g]) for jb in range(4)]
      for q, r0 in rows + ([(40, 128)] if g == 0 else []):
        for a, (scale, dst) in enumerate(zip(scales, dsts)):
          for h in (0, 8):
            dst[16 * q + h:16 * q + h + 8, :] = res[r0 + h:r0 + h + 8, _lanes(a)] * scale
    return marks

  def first_stage(i, means, marks):
    rstds, marks = [], iter(marks)
    for a in range(2):
      squares = []

      def load(slices):
        mean = after(means[a], next(marks))
        xc = [xt[2 * i + a, rows, :] - mean for rows in slices]
        squares.append(_tree_sum([v * v for v in xc]))
        return [v * modb[1, rows, :] for v, rows in zip(xc, slices)]

      radix10(rhs_v.at[i % 2, a], load)
      var = jnp.sum(_tree_sum(squares), axis=0, keepdims=True) * (1.0 / D)
      rstds.append(jnp.broadcast_to(lax.rsqrt(var + EPS), (8, 128)))
    return rstds

  def second_stage(i, rstds):
    return length64([rhs_v.at[i % 2, a] for a in range(2)], rstds,
                    [z_v.at[2 * i + a] for a in range(2)])

  wait("x0")
  means, _ = transpose_tiles(0)
  wait("x1")
  ahead, marks = transpose_tiles(1)
  rstds, means = first_stage(0, means, [None] * 6 + marks), ahead
  for i in range(NT // 2 - 2):
    if f"x{i + 2}" in groups:
      wait(f"x{i + 2}")
    marks = second_stage(i, rstds)
    ahead, more = transpose_tiles(i + 2)
    rstds, means = first_stage(i + 1, means, [None] * 2 + marks + more), ahead
  marks = second_stage(NT // 2 - 2, rstds)
  second_stage(NT // 2 - 1, first_stage(NT // 2 - 1, means, [None] * 6 + marks))

  shift_masks = [((lane >> i) & 1) == 1 for i in range(4)]

  def shuffle_filter(m, pin=None):
    pin = None if pin is None else pltpu.bitcast(pin, u32)
    for a, w_v in enumerate((wr_v, wi_v)):
      cur = [None] * 16
      for t in range(16):
        if m < 20:
          word = pltpu.bitcast(w_v[16 * m:16 * m + 16, _lanes(t)], u32)
        else:
          word = jnp.broadcast_to(w_v[KD - 1:KD, _lanes(t)].astype(f32), (8, 128))
          word = pltpu.bitcast(word, u32)
        cur[(-t) % 16] = pltpu.roll(word, t, 1) if t else after(word, pin)
      for i in range(4):
        cur = [jnp.where(shift_masks[i], cur[(j - (1 << i)) % 16], cur[j]) for j in range(16)]
      for k1 in range(16):
        wsh[a, k1, 8 * m:8 * m + 8, :] = cur[k1]

  def filter_rows(a, k1, jb):
    rows = []
    for i in range(5):
      word = wsh[a, k1, pl.ds(40 * jb + i, 8, stride=5), :]
      rows.append(pltpu.bitcast(word << 16, f32))
      rows.append(pltpu.bitcast(word & np.uint32(0xFFFF0000), f32))
    if jb == 3:
      rows.append(pltpu.bitcast(wsh[a, k1, 160:168, :], f32))
    return jnp.stack(rows, axis=0)

  def spectral(jb, c, pins):
    n = 11 if jb == 3 else 10
    rows = slice(160 * jb, 160 * jb + 16 * n)

    def load(t):
      z = z_v[t, rows, :].reshape(n, 16, 128)
      return z[:, 0:8], z[:, 8:16]

    def pinned(t):
      return [jnp.stack([after(v[q], pins[q * len(pins) // n]) for q in range(n)], axis=0)
              if pins else v for v in load(t)]

    inner = [_twiddle16(_dft4_output([pinned(b)] + [load(4 * a + b) for a in (1, 2, 3)], c), b * c)
             for b in range(4)]
    back, marks = [], []
    for e, (ar, ai) in enumerate(_dft4(inner)):
      k1 = c + 4 * e
      fr, fi = fs_v[k1, 0], fs_v[k1, 1]
      lhs = jnp.concatenate([ar, ai], axis=1).reshape(16 * n, 128).astype(bf16)
      p = jnp.dot(lhs, jnp.concatenate([fr, fi], axis=1), preferred_element_type=f32)
      marks += [p[0:8, 0:128], p[80:88, 0:128]]
      p = p.reshape(n, 16, 256)
      x = (p[:, 0:8, 0:128] - p[:, 8:16, 128:256], p[:, 0:8, 128:256] + p[:, 8:16, 0:128])
      if k1 == 0:
        shift = shift_v[rows, :].reshape(n, 16, 128)
        x = (x[0] + shift[:, 0:8], x[1] + shift[:, 8:16])
      y = jnp.concatenate(_cmul(x, (filter_rows(0, k1, jb), filter_rows(1, k1, jb))), axis=1)
      y = y.reshape(16 * n, 128).astype(bf16)
      p = lax.dot_general(y, jnp.concatenate([fr, fi], axis=0), _NT_DIMS,
                          preferred_element_type=f32)
      p = p.reshape(n, 16, 256)
      back.append((p[:, 0:8, 0:128] + p[:, 8:16, 128:256],
                   p[:, 8:16, 0:128] - p[:, 0:8, 128:256]))
    turned = [_twiddle16(v, b * c) for b, v in enumerate(_dft4(_swap(back)))]
    for b, (tr, ti) in enumerate(_swap(turned)):
      t_v[b, c, rows, :] = jnp.concatenate([tr, ti], axis=1).reshape(16 * n, 128)
    return marks

  wait("filter0")
  shuffle_filter(0)
  marks = to_columns(modulation(0), modb.at[0])
  shuffle_filter(1, marks[0])
  shuffle_filter(2, marks[4])
  radix10(rhs_v.at[0, 0], lambda slices: [modb[0, rows, :] for rows in slices])
  marks = length64([rhs_v.at[0, 0]], [jnp.where(lane == 0, float(S), 0.0)], [shift_v])
  shuffle_filter(3, marks[0])
  shuffle_filter(4, marks[6])
  ready = []
  for jb, needed in enumerate(("filter1", "filter2", None, "mod")):
    if needed:
      wait(needed)
      marks = []
    todo = list(range(5 * jb + 5, 5 * jb + 10 + (jb == 2))) if jb < 3 else []
    for c in range(4):
      marks = spectral(jb, c, marks[0:6])
      for m, mark in zip(todo[c::4], marks[0::4]):
        shuffle_filter(m, mark)
      if jb == 3:
        for j, row in ready:
          to_columns(row, modb.at[j // ND, _lanes(j % ND)])
        ready = [(j, modulation_tile(j, mark))
                 for j, mark in zip(range(2 * ND + 4 * c, 5 * ND), marks[0::2])]

  def inverse_d(b, g, pin):
    def last_radix4(q, pin):
      z = [(t_v[b, c, 16 * q:16 * q + 8, :], t_v[b, c, 16 * q + 8:16 * q + 16, :])
           for c in range(4)]
      z[0] = after(z[0][0], pin), after(z[0][1], pin)
      return _swap(_dft4(_swap(z)))

    blocks = []
    for rho in _GROUP_RES[g]:
      for jb in range(4):
        z = last_radix4(10 * jb + rho, pin)
        if rho == 0 and jb == 0:
          z = [(r, jnp.where(sub == 0, top[0], i)) for (r, i), top in zip(z, last_radix4(40, None))]
        blocks.append(jnp.concatenate([jnp.concatenate(p, axis=0) for p in z], axis=1))
    rhs = jnp.concatenate(blocks, axis=0).astype(bf16)
    y = jnp.dot(gd_v[g], rhs, preferred_element_type=f32)
    for a in range(TPC):
      z_v[4 * a + b, _lanes(g), :] = y[:, _lanes(a)]
    return y

  def residual(b):
    pin = yield
    for a in range(TPC):
      t = 4 * a + b
      sums = []
      for r8 in range(8):
        ab = [(z_v[t, 128 * g + 16 * r8:128 * g + 16 * r8 + 8, :],
               z_v[t, 128 * g + 16 * r8 + 8:128 * g + 16 * r8 + 16, :]) for g in range(5)]
        ev = _irdft5(after(ab[0][0], pin), ab[4][0], ab[4][1], ab[2][0], ab[2][1])
        od = _irdft5(ab[0][1], ab[1][0], ab[1][1], ab[3][0], ab[3][1])
        part = []
        for k in range(5):
          for d1, y in ((2 * k, ev[k] + od[k]), ((5 + 2 * k) % 10, ev[k] - od[k])):
            rows = slice(64 * d1 + 8 * r8, 64 * d1 + 8 * r8 + 8)
            x1 = xt[t, rows, :] + modb[2, rows, :] * y
            x1_v[t, rows, :] = x1
            part.append(x1)
        sums.append(_tree_sum(part))
        if r8 == 7:
          mean = jnp.sum(_tree_sum(sums), axis=0, keepdims=True) * (1.0 / D)
          mean_v[t] = jnp.broadcast_to(mean, (8, 128))
        pin = yield sums[-1]

  def inverse_std(t, mean):
    sums = []
    for r0 in range(0, D // 8, 8):
      xc = [x1_v[t, 8 * r:8 * r + 8, :] - mean for r in range(r0, r0 + 8)]
      sums.append(_tree_sum([v * v for v in xc]))
    var = jnp.sum(_tree_sum(sums), axis=0, keepdims=True) * (1.0 / D)
    return jnp.broadcast_to(lax.rsqrt(var + EPS), (8, 128))

  def normalize(b):
    pin = yield
    for p in range(2):
      tiles = [4 * a + b for a in (p, p + 2)]
      means, rstds = [], []
      for t in tiles:
        means.append(after(mean_v[t], pin))
        rstds.append(inverse_std(t, means[-1]))
        pin = yield rstds[-1]

      def rows16(k, r, scale):
        return jnp.concatenate(
            [(x1_v[tiles[k], rows, :] - means[k]) * scale * modb[4, rows, :] + modb[3, rows, :]
             for rows in (slice(r, r + 8), slice(r + 8, r + 16))], axis=0)

      for r0 in range(0, 256, 64):
        s0, s1 = after(rstds[0], pin), after(rstds[1], pin)
        for r in range(r0, r0 + 64, 16):
          quads = rows16(0, r, s0), rows16(1, r, s1), rows16(0, 256 + r, s0), rows16(1, 256 + r, s1)
          for i, v in enumerate(_strassen_right(*quads)):
            h_v[i, p, r:r + 16, :] = v.astype(bf16)
        pin = yield v[0:8]
      for k in range(2):
        scale = after(rstds[k], pin)
        for r in range(0, 128, 16):
          h5_v[p + 2 * k, r:r + 16, :] = rows16(k, 512 + r, scale).astype(bf16)
      pin = yield

  def prepare_w2():
    pin = yield
    for k in range(KT):
      w = min(128, FH - 128 * k)
      for j in range(ND):
        flipped = []
        for half in range(2):
          blk = w2_v[FH * half + 128 * k:FH * half + 128 * k + w, _lanes(j)].astype(f32)
          flipped.append(jnp.concatenate([after(blk[0:8], pin), blk[8:]], axis=0).T)
        quads = flipped[0][0:64], flipped[1][0:64], flipped[0][64:128], flipped[1][64:128]
        for i, v in enumerate(_strassen_left(*quads)):
          d_v[i, k, 64 * j:64 * j + 64, 0:w] = v.astype(bf16)
        pin = yield

  def mlp_up(r1, blocks, tick, prepare=False):
    right = [jnp.concatenate([h_v[i, p] for p in range(2)], axis=1) for i in range(7)]
    right5 = jnp.concatenate([h5_v[a] for a in range(TPC)], axis=1)
    for size in blocks:
      r0, r1 = r1, r1 + size
      top, bottom = slice(r0, r1), slice(FH + r0, FH + r1)
      if prepare:
        quads = [w1t_v[rows, c:c + 256].astype(f32) for rows in (top, bottom) for c in (0, 256)]
        left = [v.astype(bf16) for v in _strassen_left(*quads)]
        for i, v in enumerate(left):
          for k in range(2):
            u_v[i, k, top, :] = v[:, _lanes(k)]
      else:
        left = [jnp.concatenate([u_v[i, k, top, :] for k in range(2)], axis=1) for i in range(7)]
      extra = [tick(jnp.dot(w1t_v[rows, 512:D], right5, preferred_element_type=f32))
               for rows in (top, bottom)]
      quads = _strassen_result([tick(jnp.dot(a, b, preferred_element_type=f32))
                                for a, b in zip(left, right)])
      acts = []
      for q in range(4):
        u = quads[q] + extra[q // 2][:, 256 * (q % 2):256 * (q % 2) + 256]
        bias = b1b[(top, bottom)[q // 2], :]
        r = jnp.maximum(u + jnp.concatenate([bias, bias], axis=1), 0.0)
        acts.append(r * r)
      for i, v in enumerate(_strassen_right(*acts)):
        for p in range(2):
          at_v[i, p, top, :] = v[:, _lanes(p)].astype(bf16)

  def mlp_down(b, tick, done=None):
    right = [jnp.concatenate([at_v[i, p] for p in range(2)], axis=1) for i in range(7)]
    for block in DOWN_BLOCKS:
      rows = slice(64 * block[0], 64 * block[-1] + 64)
      left = [jnp.concatenate([d_v[i, k, rows, 0:min(128, FH - 128 * k)] for k in range(KT)],
                              axis=1) for i in range(7)]
      quads = _strassen_result([tick(jnp.dot(p, q, preferred_element_type=f32))
                                for p, q in zip(left, right)])
      for n, j in enumerate(block):
        for a in range(TPC):
          t = 4 * a + b
          o = jnp.concatenate([quads[q][64 * n:64 * n + 64, _lanes(a % 2)]
                               for q in (a // 2, 2 + a // 2)], axis=0)
          res = x1_v[t, _lanes(j), :] + modb[5, _lanes(j), :] * (o + b2b[_lanes(j), :])
          o_v[_tile_rows(t), _lanes(j)] = res.astype(bf16).T
        if done:
          done(j)

  def out_copy(t, cols):
    return pltpu.make_async_copy(o_v.at[_tile_rows(t), cols], out_hbm.at[0, _tile_rows(t), cols],
                                 out_sem)

  piece = lambda side: functools.partial(_step, side)

  res, norm = _begin(residual(0)), _begin(normalize(0))
  done, count = [None] * 3, 0
  for b in range(NCH):
    for g in range(5):
      y = inverse_d(b, g, done[-3])
      if (b, g) == (0, 1):
        for j, row in ready:
          to_columns(row, modb.at[j // ND, _lanes(j % ND)])
      last = y[0:8, 0:128]
      for r in range(3 if b > 0 else 0):
        out = _step(res if count < 8 * TPC else norm, y[32 * r:32 * r + 8, 0:128])
        last = last if out is None else out
        count += 1
      done.append(last)
  _finish(res)
  _finish(norm)

  wait("w1")
  res = _begin(residual(1))
  mlp_up(0, [32] * 6, _Paced((2, piece(res))), prepare=True)
  wait("w2")
  flip = _begin(prepare_w2())
  gate = modulation(5)
  mlp_up(192, [32] * 21,
         _Paced((30, piece(res)), (5, piece(flip)), (F, lambda _: to_columns(gate, modb.at[5]))),
         prepare=True)
  _finish(flip)
  _finish(res)

  def chunk(b, carry):
    norm = _begin(normalize(b + 1))
    _step(norm, None)
    mlp_down(b, _Paced((1, piece(norm))))
    _finish(norm)
    res = _begin(residual(jnp.minimum(b + 2, NCH - 1)))
    mlp_up(0, UP_BLOCKS, _Paced((2, piece(res))))
    _finish(res)
    for a in range(TPC):
      out_copy(4 * a + b, slice(None)).start()
    return carry

  lax.fori_loop(0, NCH - 1, chunk, 0)

  early, late = slice(0, 128 * (ND - 1)), slice(128 * (ND - 1), D)

  def send_early(j):
    if j == ND - 2:
      for a in range(TPC):
        out_copy(4 * a + NCH - 1, early).start()

  mlp_down(NCH - 1, _Paced(), send_early)
  for a in range(TPC):
    out_copy(4 * a + NCH - 1, late).start()
  for t in range(NT):
    out_copy(t, early if t % 4 == NCH - 1 else slice(None)).wait()
  for a in range(TPC):
    out_copy(4 * a + NCH - 1, late).wait()


@jax.jit
def pallas_adaLN_cond__spectral_gfnet__dense_activation_squared_relu__prompt_kernel(
    A_x: jax.Array,
    A_w_r: jax.Array,
    A_w_i: jax.Array,
    B_x: jax.Array,
    B_w1: jax.Array,
    B_b1: jax.Array,
    B_w2: jax.Array,
    B_b2: jax.Array,
    c: jax.Array,
    w_mod: jax.Array,
):
  del B_x
  vmem = pltpu.VMEM
  operands = (A_x, A_w_r.T, A_w_i.T, B_w1.T, B_b1, B_w2, B_b2, c, w_mod, _FD, _GD)
  scratch = [
      vmem((NT, 128, D), bf16), vmem((KD, S), bf16), vmem((KD, S), bf16),
      vmem((F, D), bf16), vmem((F,), bf16), vmem((F, D), bf16), vmem((D,), bf16),
      vmem((1, D), bf16), vmem((6 * ND, D, 128), bf16),
      vmem((5, 144, 128), bf16), vmem((5, 128, 128), bf16), vmem((16, 2, 128, 128), bf16),
      vmem((6, D, 128), f32), vmem((D, 128), f32),
      vmem((F, 128), f32), vmem((D, 128), f32),
      vmem((NT, D, 128), f32),
      vmem((2, 2, 5, 128, 128), bf16),
      vmem((656, 128), f32),
      vmem((NT, 656, 128), f32),
      vmem((NCH, 4, 656, 128), f32),
      vmem((2, 16, 168, 128), u32),
      vmem((NT, D, 128), f32), vmem((NT, 8, 128), f32),
      vmem((7, 2, 256, 128), bf16), vmem((TPC, 128, 128), bf16),
      vmem((7, 2, FH, 128), bf16),
      vmem((7, 2, FH, 128), bf16),
      vmem((7, KT, D // 2, 128), bf16),
      vmem((S, D), bf16),
      pltpu.SemaphoreType.DMA((14,)), pltpu.SemaphoreType.DMA,
  ]
  return pl.pallas_call(
      _kernel,
      out_shape=jax.ShapeDtypeStruct(A_x.shape, A_x.dtype),
      in_specs=[pl.BlockSpec(memory_space=pl.ANY)] * len(operands),
      out_specs=pl.BlockSpec(memory_space=pl.ANY),
      scratch_shapes=scratch,
      compiler_params=pltpu.CompilerParams(vmem_limit_bytes=100 * 2**20),
      name="adaln_gfnet_mlp",
  )(*operands)
```
